```python
import jax
import jax.numpy as jnp

def _softmax(x, axis=-1):
    return jax.nn.softmax(x, axis=axis)
def _gelu(x):
    return jax.nn.gelu(x, approximate=True)
def _silu(x):
    return jax.nn.silu(x)
def _sigmoid(x):
    return jax.nn.sigmoid(x)
def _layernorm(x, axis=-1, eps=1e-5):
    m = jnp.mean(x, axis=axis, keepdims=True)
    v = jnp.var(x, axis=axis, keepdims=True)
    return (x - m) / jnp.sqrt(v + eps)
def _scatter_add(tgt, idx, src, axis=0):
    return tgt.at[idx].add(src)
def _segment_sum(src, seg, n):
    return jax.ops.segment_sum(src, seg, n)
class _Rng:
    def __init__(self, key):
        self._k = key
    def _next(self):
        self._k, sub = jax.random.split(self._k)
        return sub
    def normal(self, shape):
        return jax.random.normal(self._next(), shape, dtype=jnp.bfloat16)
    def randint(self, lo, hi, shape):
        return jax.random.randint(self._next(), shape, lo, hi, dtype=jnp.int32)
    def uniform(self, shape, lo=0.0, hi=1.0):
        return jax.random.uniform(self._next(), shape, jnp.bfloat16, lo, hi)
    def permutation(self, n):
        return jax.random.permutation(self._next(), n)


kernel_name = 'standalone__mha_softmax__near_ridge'

def _fwd_setup_inputs():
    _rng = _Rng(jax.random.key(int.from_bytes(__import__("os").urandom(4), "little")))
    _w = (lambda a: (lambda t: t.astype(jnp.bfloat16) if jnp.issubdtype(t.dtype, jnp.floating) else t)(jnp.asarray(a)))
    B, H, Sq, Sk, D = 16, 32, 384, 1024, 128
    return {
        "q": _w((lambda *s: _rng.normal(s) * 0.05)(B, H, Sq, D)),
        "k": _w((lambda *s: _rng.normal(s) * 0.05)(B, H, Sk, D)),
        "v": _w((lambda *s: _rng.normal(s) * 0.05)(B, H, Sk, D)),
    }

def _fwd_reference(q, k, v):
    scale = q.shape[-1] ** -0.5
    scores = jnp.einsum("bhqd,bhkd->bhqk", q, k) * scale
    p = _softmax(scores, axis=-1)
    return jnp.einsum("bhqk,bhkd->bhqd", p, v)


def setup_inputs():
    _inp = _fwd_setup_inputs()
    _gk = jax.random.fold_in(jax.random.key(int.from_bytes(__import__("os").urandom(4), "little")), 2**31 - 1)
    _shapes = [[16, 32, 384, 128]]
    _dtypes = ['bfloat16']
    _gks = jax.random.split(_gk, len(_shapes))
    _gs = [jax.random.normal(k, s, dtype=jnp.dtype(d)) * 0.05 for k, s, d in zip(_gks, _shapes, _dtypes)]
    _inp["grad_out"] = _gs[0]
    return _inp

def reference(q, k, v, grad_out):
    _const = dict()
    def _f(*_d):
        return _fwd_reference(**{'q': _d[0], 'k': _d[1], 'v': _d[2], **_const})
    _out, _vjp = jax.vjp(_f, q, k, v)
    _grads = _vjp(grad_out)
    _out0 = jnp.asarray(_out)
    return (_out0, *[jnp.asarray(_g) for _g in _grads])
```

```python
import functools, math
import jax, jax.numpy as jnp
import jax.experimental.pallas as pl
import jax.experimental.pallas.tpu as pltpu
NT = (((1,), (1,)), ((), ()))
NN = (((1,), (0,)), ((), ()))
f32 = jnp.float32; bf16 = jnp.bfloat16; u32 = jnp.uint32; i32 = jnp.int32
def dot(a, b, dn=NN):
    return jax.lax.dot_general(a, b, dn, preferred_element_type=f32)
T = 128
def tsum(xs): return functools.reduce(jnp.add, xs)

def make(hb=8, ck=256, pro="S0 S1 S2 X0 O0 V0 P0 X1 O1 K0 Q0 P1 V1 K1 Q1 X2", body="O0 S1 P0 V0 K0 Q0 X1", epi="O0 Q1 P0 V0 Q0 K0",
         nb=3, xt=False, pace=(0, 999), pace0=(0, 999), gx=128, tieout=True, marg=16, nobc=True, zmode=1):
    @jax.jit
    def fn(q, k, v, g):
        B, H, Sq, D = q.shape; Sk = k.shape[2]; BH = B * H
        scale = D ** -0.5
        c = scale * math.log2(math.e)
        nj = Sq // T; nc = Sk // ck; nt = Sk // T; tpc = ck // T
        names = []
        for nm, cnt, packed in [("s", nb, 0), ("e", nb, 1), ("d", nb, 1), ("ak", 2, 0), ("av", 2, 0), ("tk", 2, 1), ("tv", 2, 1)]:
            for b in range(cnt):
                for i in range(nt): names.append((nm, b, i, packed))
        scratch = [pltpu.VMEM((T, T), bf16 if p else f32) for (_, _, _, p) in names]
        def kern(z_ref, q_ref, k_ref, v_ref, g_ref, o_ref, dq_ref, dk_ref, dv_ref, *scr):
            sc = {n[:3]: (r, n[3]) for n, r in zip(names, scr)}
            z = z_ref[0] if zmode == 0 else jax.lax.shift_right_logical(pl.program_id(0), 24)
            zv = jnp.full((8, T), z, i32)
            U = hb * nj
            st = [dict() for _ in range(U)]
            toks = []; pend = []
            def tie(m8, x):
                return pltpu.bitcast(pltpu.bitcast(m8, i32) | (pltpu.bitcast(x, i32) & zv), f32)
            def addtoks(x):
                toks.extend(x[r * 8:(r + 1) * 8] for r in range(x.shape[0] // 8))
            def rows(ref, h, i, n):
                return pltpu.bitcast(ref.bitcast(u32)[h, i * n // 2:(i + 1) * n // 2, :], bf16)
            def put(ref, h, i, n, x): ref[h, i * n:(i + 1) * n, :] = x
            def sput(nm, b, r0, x):
                for o in range(0, x.shape[0], T):
                    n = min(T, x.shape[0]); ti, oo = divmod(r0 + o, T); r, p = sc[nm, b, ti]
                    y = x[o:o + n]
                    if nm[0] == "t": r.bitcast(u32)[oo // 2:(oo + n) // 2, :] = pltpu.bitcast(y, u32)
                    else: r[oo:oo + n, :] = y.astype(r.dtype)
            def sget(nm, b, r0, n):
                xs = []
                for o in range(r0, r0 + n, T):
                    ti, oo = divmod(o, T); r, p = sc[nm, b, ti]; nn = min(n, T)
                    if p: oo, nn, r = oo // 2, nn // 2, r.bitcast(u32)
                    xs.append(r[pl.ds(pl.multiple_of(z + oo, 8), nn), :])
                x = xs[0] if len(xs) == 1 else jnp.concatenate(xs, axis=0)
                return pltpu.bitcast(x, bf16) if p else x
            def S(u):
                h, j = divmod(u, nj); s = st[u]; b = u % nb
                qs = (rows(q_ref, h, j, T).astype(f32) * c).astype(bf16)
                ms = []
                for i in range(nc):
                    x = dot(rows(k_ref, h, i, ck), qs, NT)
                    if i == 0: addtoks(x)
                    sput("s", b, i * ck, x)
                    ms.append(x.reshape(ck // 8, 8, T).max(0))
                m = jnp.max(functools.reduce(jnp.maximum, ms), axis=0, keepdims=True)
                s["m"] = jnp.broadcast_to(m, (8, T)); s["t0"] = len(toks)
            def X(u):
                s = st[u]; b = u % nb
                ls = []; ng = Sk // gx; p0, p1 = pace0 if u == 0 else pace
                p1 = min(p1, len(toks) - s['t0'] - marg); p0 = max(p0, len(toks) - s['t0'] - 128)
                for i in range(ng):
                    m = s["m"]
                    ti = s["t0"] + p0 + (p1 - p0) * i // ng
                    if p1 > p0 and i > 0 and ti < len(toks): m = tie(m, toks[ti])
                    if i == ng - 1:
                        while pend and pend[0][0] <= len(toks) - 64: m = tie(m, pend.pop(0)[1])
                    e = jnp.exp2(sget("s", b, i * gx, gx).reshape(gx // 8, 8, T) - m[None])
                    sput("e", b, i * gx, e.reshape(gx, T))
                    ls.append(e.sum(0))
                s["r"] = 1.0 / jnp.sum(tsum(ls), axis=0, keepdims=True)
            def tr(src, nm, h, j):
                if not xt: return [rows(src, h, i, T).T for i in range(nt)]
                if j == 0:
                    for i in range(nt): sput(nm, h % 2, i * T, rows(src, h, i, T).T)
                return [sget(nm, h % 2, i * T, T) for i in range(nt)]
            def tdot(ts, nm, b):
                ps = [dot(ts[i], sget(nm, b, i * T, T)) for i in range(nt)]
                addtoks(ps[0]); addtoks(ps[nt // 2])
                return tsum(ps)
            def outT(ref, h, j, x):
                x = x.T
                if tieout: pend.append((len(toks), x[T - 8:]))
                put(ref, h, j, T, x.astype(bf16))
            def O(u):
                h, j = divmod(u, nj); s = st[u]; b = u % nb
                ot = tdot(tr(v_ref, "tv", h, j), "e", b) * s["r"]
                gt = rows(g_ref, h, j, T).astype(f32).T
                s["delta"] = jnp.sum(gt * ot, axis=0, keepdims=True)
                s["gr"] = (gt * s["r"]).astype(bf16)
                outT(o_ref, h, j, ot)
            def acc(an, out_ref, u, ln, w):
                h, j = divmod(u, nj); b = u % nb
                for i in range(nc):
                    x = dot(sget(ln, b, i * ck, ck), w, NT)
                    if i == 0: addtoks(x)
                    if j > 0: x = x + sget(an, (j - 1) % 2, i * ck, ck)
                    if j == nj - 1: put(out_ref, h, i, ck, x.astype(bf16))
                    else: sput(an, j % 2, i * ck, x)
            def V(u): acc("av", dv_ref, u, "e", st[u]["gr"])
            def P(u):
                h, j = divmod(u, nj); s = st[u]; b = u % nb
                gj = rows(g_ref, h, j, T)
                for i in range(nc):
                    p = dot(rows(v_ref, h, i, ck), gj, NT)
                    if i == 0: addtoks(p)
                    sput("d", b, i * ck, sget("e", b, i * ck, ck).astype(f32) * (p - s["delta"]))
            def K(u):
                h, j = divmod(u, nj); s = st[u]
                qt = rows(q_ref, h, j, T).astype(f32).T
                acc("ak", dk_ref, u, "d", (qt * (s["r"] * scale)).astype(bf16))
            def Q(u):
                h, j = divmod(u, nj); s = st[u]; b = u % nb
                dqt = tdot(tr(k_ref, "tk", h, j), "d", b)
                outT(dq_ref, h, j, dqt * (s["r"] * scale))
            F = dict(S=S, X=X, O=O, V=V, P=P, K=K, Q=Q)
            seq = [(t[0], int(t[1:])) for t in pro.split()]
            ep = [(t[0], U - 1 - int(t[1:])) for t in epi.split()]
            for t in range(-2, U + 1):
                for tok in body.split():
                    it = (tok[0], t + int(tok[1:]))
                    if 0 <= it[1] < U and it not in seq and it not in ep: seq.append(it)
            seq += ep
            assert len(set(seq)) == len(seq) == 7 * U
            for n, u in seq: F[n](u)
        qs = pl.BlockSpec((hb, Sq, D), lambda i, z: (i, 0, 0))
        ks = pl.BlockSpec((hb, Sk, D), lambda i, z: (i, 0, 0))
        sq = jax.ShapeDtypeStruct((BH, Sq, D), bf16); sk = jax.ShapeDtypeStruct((BH, Sk, D), bf16)
        o, dq, dk, dv = pl.pallas_call(kern,
            grid_spec=pltpu.PrefetchScalarGridSpec(num_scalar_prefetch=1, grid=(BH // hb,), in_specs=[qs, ks, ks, qs],
                out_specs=[qs, qs, ks, ks], scratch_shapes=scratch),
            out_shape=[sq, sq, sk, sk],
            compiler_params=pltpu.CompilerParams(dimension_semantics=("parallel",), vmem_limit_bytes=100*1024*1024, disable_bounds_checks=nobc),
        )(jnp.zeros((1,), jnp.int32), q.reshape(BH, Sq, D), k.reshape(BH, Sk, D), v.reshape(BH, Sk, D), g.reshape(BH, Sq, D))
        return o.reshape(q.shape), dq.reshape(q.shape), dk.reshape(k.shape), dv.reshape(k.shape)
    return fn


pallas_standalone__mha_softmax__near_ridge_kernel = jax.jit(lambda q, k, v, grad_out: make()(q, k, v, grad_out))
```

```python
import functools, math
import jax, jax.numpy as jnp
import jax.experimental.pallas as pl
import jax.experimental.pallas.tpu as pltpu
NT = (((1,), (1,)), ((), ()))
NN = (((1,), (0,)), ((), ()))
f32 = jnp.float32; bf16 = jnp.bfloat16; u32 = jnp.uint32; i32 = jnp.int32
def dot(a, b, dn=NN):
    return jax.lax.dot_general(a, b, dn, preferred_element_type=f32)
T = 128; HT = 64
def tsum(xs): return functools.reduce(jnp.add, xs)
def bcomb(b00, b01, b10, b11): return [b00 + b11, b00, b01 - b11, b10 - b00, b11, b00 + b01, b10 + b11]
def acomb(a00, a01, a10, a11): return [a00 + a11, a10 + a11, None, None, a00 + a01, a10 - a00, a01 - a11]
def ccomb(g00, g01, g10, g11): return [g00 + g11, g10 - g11, g01 + g11, g00 + g10, g01 - g00, g11, g00]
PRO = "Sc0 Tv0@1 Sa0 Xs0@1 Sb0 La0@1 Cg0@1 Sa1 Lb0@1 Os0 Sb1 Sc1 Ps0 Xp0@4/2 Av0@4/2 Tk0@3"
HEAD = "Os0 Sa1 Sb1 Sc1 Ps0 Xp0@5/2 Tk0@4"
REST = "Op0 La1@1 Cq0@1 Tv1@1 V0 Lb1@1 Pp0 Qs0 Ak0@1 K0 Xs1@1 Qp0 Cg1@1/2 Av1@1"
LAST = "Os0 Ps0 Xp0@5/2 Op0 Tk0@1 V0 Cq0@1 Ak0@1 Pp0 Qs0 F Ky0 Qp0 Kz0"

HB = 8
GX = 16
GL = 32
LAG = 80


@jax.jit
def pallas_standalone__mha_softmax__near_ridge_kernel(q, k, v, grad_out):
    g = grad_out; hb, gx, gl, lag, kt = HB, GX, GL, LAG, 224
    B, H, Sq, D = q.shape; Sk = k.shape[2]; BH = B * H
    scale = D ** -0.5
    c = scale * math.log2(math.e)
    ck = 256; nc = 4; KH = Sk // 2
    names = []
    for par in range(2):
        names += [(("s", par, j, i), ck, f32) for j in range(3) for i in range(nc)]
        for i in range(4):
            names += [(("pp", par, i), 9 * T, bf16), (("ps", par, i), ck, bf16), (("dp", par, i), 7 * T, bf16), (("ds", par, i), ck, bf16),
                      (("av", par, i), 4 * HT, bf16), (("ak", par, i), 4 * HT, bf16), (("avc", par, i), 5 * HT, bf16), (("akc", par, i), 5 * HT, bf16)]
        names += [(("cg", par), 13 * HT, bf16), (("cq", par), 9 * HT, bf16)]
    scratch = [pltpu.VMEM((n, T), dt) for (_, n, dt) in names]
    def kern(q_ref, k_ref, v_ref, g_ref, o_ref, dq_ref, dk_ref, dv_ref, *scr):
        sc = {n[0]: r for n, r in zip(names, scr)}
        z = jax.lax.shift_right_logical(pl.program_id(0), 24)
        zv = jnp.full((8, T), z, i32)
        st = [dict() for _ in range(hb)]
        toks = []; marks = []; win = [0, 0]; pend = []; fin = []
        def drain(x):
            if not (fin and pend and pend[0][0] <= len(toks) - lag): return x
            y = pltpu.bitcast(x[:8], i32)
            while pend and pend[0][0] <= len(toks) - lag: y = y | (pltpu.bitcast(pend.pop(0)[1], i32) & zv)
            return jnp.concatenate([pltpu.bitcast(y, u32), x[8:]], axis=0)
        def tie(m8, f):
            if win[1] <= win[0]: return m8
            ti = min(win[0] + int((win[1] - win[0]) * f), len(toks) - 1); x, r = toks[ti]
            y = pltpu.bitcast(m8, i32) | (pltpu.bitcast(x[r * 8:r * 8 + 8], i32) & zv)
            return pltpu.bitcast(y, m8.dtype)
        def addtoks(x): toks.extend((x, r) for r in range(x.shape[0] // 8))
        def rows(ref, h, r0, n, f=None, dep=False):
            x = ref.bitcast(u32)[h, r0 // 2:(r0 + n) // 2, :]
            if f is not None: x = jnp.concatenate([tie(x[:8], f), x[8:]], axis=0)
            return pltpu.bitcast(drain(x) if dep else x, bf16)
        def sput(key, r0, x):
            r = sc[key]
            if x.dtype == bf16: r.bitcast(u32)[r0 // 2:(r0 + x.shape[0]) // 2, :] = pltpu.bitcast(x, u32)
            else: r[r0:r0 + x.shape[0], :] = x.astype(r.dtype)
        def sget(key, r0, n, dep=False):
            r = sc[key]
            if r.dtype == f32: return r[pl.ds(pl.multiple_of(z + r0, 8), n), :]
            x = r.bitcast(u32)[pl.ds(pl.multiple_of(z + r0 // 2, 8), n // 2), :]
            return pltpu.bitcast(drain(x) if dep else x, bf16)
        def outT(ref, h, r0, x):
            y = pltpu.bitcast(x.astype(bf16).T, u32)
            pend.append((len(toks), y[HT - 8:]))
            ref.bitcast(u32)[h, r0 // 2:(r0 + T) // 2, :] = y
        def colsum(x): return jnp.sum(x, axis=0, keepdims=True)
        def S(h, j):
            qs = rows(q_ref, h, j * T, T)
            ms = []
            for i in range(nc):
                x = dot(rows(k_ref, h, i * ck, ck, dep=True), qs, NT)
                if i == 0: addtoks(x)
                x = x * c
                sput(("s", h % 2, j, i), 0, x)
                ms.append(x.reshape(ck // 8, 8, T).max(0))
            m = jnp.max(functools.reduce(jnp.maximum, ms), axis=0, keepdims=True)
            st[h]["m", j] = jnp.broadcast_to(m, (8, T))
        def ex(h, j, r0, n, m):
            s = sget(("s", h % 2, j, r0 // ck), r0 % ck, n)
            return jnp.exp2(s.reshape(n // 8, 8, T) - m[None])
        def L(h, j):
            m = st[h]["m", j]; n = Sk // gl
            ls = [ex(h, j, i * gl, gl, tie(m, i / n)).sum(0) for i in range(n)]
            st[h]["m", j] = m + jnp.log2(jnp.broadcast_to(colsum(tsum(ls)), (8, T)))
        def Xs(h):
            m = st[h]["m", 2]; n = Sk // gl; ls = []
            for i in range(n):
                e = ex(h, 2, i * gl, gl, tie(m, i / n))
                sput(("ps", h % 2, i * gl // ck), i * gl % ck, e.reshape(gl, T)); ls.append(e.sum(0))
            st[h]["r"] = 1.0 / colsum(tsum(ls))
        def Xp(h):
            m0 = st[h]["m", 0]; m1 = st[h]["m", 1]; n = KH // gx
            for t in range(n):
                ms = [tie(m0, t / n), tie(m1, t / n)]
                b = [ex(h, j, a * KH + t * gx, gx, ms[j]).reshape(gx, T) for a in range(2) for j in range(2)]
                i, o = divmod(t * gx, T)
                for r, x in enumerate(bcomb(*b) + [b[1], b[2]]): sput(("pp", h % 2, i), r * T + o, x)
        def Tr(ref, nm, h):
            for i in range(4):
                for a in range(2): sput((nm, h % 2, i), a * T, rows(ref, h, a * KH + i * T, T, (2 * i + a) / 8).T)
        def Ac(nm, h):
            for i in range(4):
                for o in range(0, HT, 16):
                    f = (i * HT + o) / (4 * HT)
                    xs = [tie(sget((nm, h % 2, i), r0 + o, 16), f).astype(f32) for r0 in (0, T, HT, T + HT)]
                    cs = [x for x in acomb(*xs) if x is not None]
                    for r, x in enumerate(cs): sput((nm + "c", h % 2, i), r * HT + o, x)
        AOFF = [("c", 0), ("c", HT), ("", 0), ("", 3 * HT), ("c", 2 * HT), ("c", 3 * HT), ("c", 4 * HT)]
        def Cmb(ref, nm, h, mul):
            ts = [rows(ref, h, j * T, T, j / 3).T.astype(f32) for j in range(3)]
            if mul is not None: ts = [x * mul for x in ts]
            cs = ccomb(ts[0][:HT], ts[1][:HT], ts[0][HT:], ts[1][HT:]) + [ts[2] * st[h]["r"]]
            if mul is None: cs += [None, ts[0][HT:], ts[1][:HT], ts[2]]
            for r, x in enumerate(cs):
                if x is not None: sput((nm, h % 2), r * HT, x)
        def fwdp(h, an, bn):
            M = {}
            for r in (2, 4, 0, 6, 3, 1, 5):
                ps = [dot(sget((an + AOFF[r][0], h % 2, i), AOFF[r][1], HT, True), sget((bn, h % 2, i), r * T, T)) for i in range(4)]
                addtoks(ps[0]); M[r] = tsum(ps)
            return [[((M[0] - M[4]) + M[6]) + M[3], M[2] + M[4]], [M[3] + M[1], ((M[2] + M[0]) - M[1]) + M[5]]]
        def fwds(h, an, bn):
            ps = [dot(sget((an, h % 2, t % 4), t // 4 * T, T, True), sget((bn, h % 2, t // 2), t % 2 * T, T)) for t in range(8)]
            addtoks(ps[0]); addtoks(ps[4])
            return tsum(ps)
        def Op(h):
            C = fwdp(h, "av", "pp")
            G = [[sget(("cg", h % 2), o * HT, HT).astype(f32) for o in row] for row in ((6, 10), (9, 5))]
            for j in range(2):
                st[h]["d", j] = colsum(G[0][j] * C[0][j] + G[1][j] * C[1][j])
                outT(o_ref, h, j * T, jnp.concatenate([C[0][j], C[1][j]], axis=0))
        def Os(h):
            ot = fwds(h, "av", "ps") * st[h]["r"]
            st[h]["d", 2] = colsum(sget(("cg", h % 2), 11 * HT, T).astype(f32) * ot)
            outT(o_ref, h, 2 * T, ot)
        def Qp(h):
            C = fwdp(h, "ak", "dp")
            for j in range(2): outT(dq_ref, h, j * T, jnp.concatenate([C[0][j], C[1][j]], axis=0) * scale)
        def Qs(h): outT(dq_ref, h, 2 * T, fwds(h, "ak", "ds") * (st[h]["r"] * scale))
        def Pp(h):
            gs = [rows(g_ref, h, j * T, T) for j in range(2)]
            for s in range(2):
                p = [dot(rows(v_ref, h, a * KH + s * ck, ck, dep=True), gs[j], NT) for a in range(2) for j in range(2)]
                addtoks(p[0])
                for u in range(2):
                    i = 2 * s + u
                    d = [sget(("pp", h % 2, i), r * T, T).astype(f32) * (p[n][u * T:(u + 1) * T] - st[h]["d", n % 2])
                         for n, r in enumerate((1, 7, 8, 4))]
                    for r, x in enumerate(bcomb(*d)): sput(("dp", h % 2, i), r * T, x)
        def Ps(h):
            g2 = rows(g_ref, h, 2 * T, T)
            for i in range(nc):
                p = dot(rows(v_ref, h, i * ck, ck, dep=True), g2, NT)
                if i == 0: addtoks(p)
                sput(("ds", h % 2, i), 0, sget(("ps", h % 2, i), 0, ck).astype(f32) * (p - st[h]["d", 2]))
        def bwd(h, cn, bn, sn, out_ref):
            cnt = 0
            for i in range(4):
                N = {}
                for r in (4, 6, "a1", 2, 0, 5, "a0", 1, 3):
                    if isinstance(r, str):
                        t = int(r[1]) * 4 + i; w = sget((sn, h % 2, t // 2), t % 2 * T, T)
                        x = dot(sget((cn, h % 2), 7 * HT, T), w, NT); js = [x[:HT], x[HT:]]
                        N[r] = js
                    else:
                        N[r] = dot(sget((cn, h % 2), r * HT, HT, True), sget((bn, h % 2, i), r * T, T), NT); js = [N[r]]
                    for x in js:
                        if cnt % 4 == 0: addtoks(x)
                        cnt += 1
                d01 = (N[4] + N[6]) + N["a1"][0]
                d00 = (((N[4] + N[2]) + N[0]) - N[5]) + N["a0"][0]
                d10 = (N[5] + N["a0"][1]) + N[1]
                d11 = (((N["a1"][1] - N[6]) + N[0]) + N[1]) + N[3]
                outT(out_ref, h, i * T, jnp.concatenate([d00, d10], axis=0))
                outT(out_ref, h, KH + i * T, jnp.concatenate([d01, d11], axis=0))
        def Ky(h):
            for i in range(4):
                N = {}
                for n, r in enumerate((4, 6, 2, 0, 5, 1, 3)):
                    N[r] = dot(sget(("cq", h % 2), r * HT, HT, True), sget(("dp", h % 2, i), r * T, T), NT)
                    if (7 * i + n) % 4 == 0: addtoks(N[r])
                lo = jnp.concatenate([((N[4] + N[2]) + N[0]) - N[5], N[5] + N[1]], axis=0)
                hi = jnp.concatenate([N[4] + N[6], ((N[0] - N[6]) + N[1]) + N[3]], axis=0)
                sput(("s", h % 2, 0, i // 2), i % 2 * T, lo.T); sput(("s", h % 2, 0, 2 + i // 2), i % 2 * T, hi.T)
        def Kz(h):
            w = sget(("cq", h % 2), 7 * HT, T)
            for i in range(nc):
                x = dot(sget(("ds", h % 2, i), 0, ck, True), w, NT); a = sget(("s", h % 2, 0, i), 0, ck)
                if i == nc - 1:
                    y = pltpu.bitcast(a[kt:kt + 8], i32)
                    while pend: y = y | (pltpu.bitcast(pend.pop(0)[1], i32) & zv)
                    a = jnp.concatenate([a[:kt], pltpu.bitcast(y, f32), a[kt + 8:]], axis=0)
                x = x + a
                dk_ref[h, i * ck:(i + 1) * ck, :] = x.astype(bf16)
        F = dict(Ky=Ky, Kz=Kz, Sa=lambda h: S(h, 0), Sb=lambda h: S(h, 1), Sc=lambda h: S(h, 2), Xs=Xs, Xp=Xp, Op=Op, Os=Os, Qp=Qp, Qs=Qs,
                 Pp=Pp, Ps=Ps, V=lambda h: bwd(h, "cg", "pp", "ps", dv_ref), K=lambda h: bwd(h, "cq", "dp", "ds", dk_ref),
                 La=lambda h: L(h, 0), Lb=lambda h: L(h, 1), Av=lambda h: Ac("av", h), Ak=lambda h: Ac("ak", h),
                 Tv=lambda h: Tr(v_ref, "av", h), Tk=lambda h: Tr(k_ref, "ak", h),
                 Cg=lambda h: Cmb(g_ref, "cg", h, None), Cq=lambda h: Cmb(q_ref, "cq", h, scale))
        done = set()
        for h0 in range(hb):
            for tok in (PRO + " " + REST if h0 == 0 else LAST if h0 == hb - 1 else HEAD + " " + REST).split():
                if tok == "F": fin.append(1); continue
                tok, _, w = tok.partition("@"); nm, h = tok[:-1], h0 + int(tok[-1])
                if h >= hb: continue
                assert (nm, h) not in done; done.add((nm, h))
                if w:
                    w, _, mg = w.partition("/")
                    win[:] = [marks[-int(w)], len(toks) - 8 * int(mg or 0)] if int(w) else [0, 0]
                else: marks.append(len(toks))
                F[nm](h)
        assert len(done) == (len(F) - 2) * hb + (("Ky", hb - 1) in done)
    qs = pl.BlockSpec((hb, Sq, D), lambda i: (i, 0, 0))
    ks = pl.BlockSpec((hb, Sk, D), lambda i: (i, 0, 0))
    sq = jax.ShapeDtypeStruct((BH, Sq, D), bf16); sk = jax.ShapeDtypeStruct((BH, Sk, D), bf16)
    o, dq, dk, dv = pl.pallas_call(kern, grid=(BH // hb,), in_specs=[qs, ks, ks, qs], out_specs=[qs, qs, ks, ks],
        scratch_shapes=scratch, out_shape=[sq, sq, sk, sk],
        compiler_params=pltpu.CompilerParams(dimension_semantics=("arbitrary",), vmem_limit_bytes=100*1024*1024, disable_bounds_checks=True),
    )(q.reshape(BH, Sq, D), k.reshape(BH, Sk, D), v.reshape(BH, Sk, D), g.reshape(BH, Sq, D))
    return o.reshape(q.shape), dq.reshape(q.shape), dk.reshape(k.shape), dv.reshape(k.shape)
```

```python
import functools, math
import jax, jax.numpy as jnp
import jax.experimental.pallas as pl
import jax.experimental.pallas.tpu as pltpu
NT = (((1,), (1,)), ((), ()))
NN = (((1,), (0,)), ((), ()))
f32 = jnp.float32; bf16 = jnp.bfloat16; u32 = jnp.uint32; i32 = jnp.int32
def dot(a, b, dn=NN):
    return jax.lax.dot_general(a, b, dn, preferred_element_type=f32)
T = 128; HT = 64
def tsum(xs): return functools.reduce(jnp.add, xs)
def bcomb(b00, b01, b10, b11): return [b00 + b11, b00, b01 - b11, b10 - b00, b11, b00 + b01, b10 + b11]
def acomb(a00, a01, a10, a11): return [a00 + a11, a10 + a11, None, None, a00 + a01, a10 - a00, a01 - a11]
def ccomb(g00, g01, g10, g11): return [g00 + g11, g10 - g11, g01 + g11, g00 + g10, g01 - g00, g11, g00]
PRO = "Sc0 Tv0@1 Sa0 Xs0@1 Sb0 La0@1 Cg0@1 Sa1 Lb0@1 Os0 Sb1 Sc1 Ps0 Xp0@4/2 Av0@4/2 Tk0@3"
HEAD = "Os0 Sa1 Sb1 Sc1 Ps0 Xp0@5/2 Tk0@4"
REST = "Op0 La1@1 Cq0@1 Tv1@1 V0 Lb1@1 Pp0 Qs0 Ak0@1 K0 Xs1@1 Qp0 Cg1@1/2 Av1@1"
LAST = "Os0 Ps0 Xp0@4/2 Tk0@2 Op0 Cq0@1 V0 Pp0 Qs0 Ak0@1 F Ky0 Qp0 Kz0"

HB = 8
GX = 16
GL = 32
LAG0 = 300
LAG = 80
CUT = (4, 6)


@jax.jit
def pallas_standalone__mha_softmax__near_ridge_kernel(q, k, v, grad_out):
    g = grad_out; hb, gx, gl, lag, lag0, cut, dat, kt = HB, GX, GL, LAG, LAG0, CUT, "Op", 224
    B, H, Sq, D = q.shape; Sk = k.shape[2]; BH = B * H
    scale = D ** -0.5
    c = scale * math.log2(math.e)
    ck = 256; nc = 4; KH = Sk // 2
    names = []
    for par in range(2):
        names += [(("s", par, j, i), ck, f32) for j in range(3) for i in range(nc)]
        for i in range(4):
            names += [(("pp", par, i), 9 * T, bf16), (("ps", par, i), ck, bf16), (("dp", par, i), 7 * T, bf16), (("ds", par, i), ck, bf16),
                      (("av", par, i), 4 * HT, bf16), (("ak", par, i), 4 * HT, bf16), (("avc", par, i), 5 * HT, bf16), (("akc", par, i), 5 * HT, bf16)]
        names += [(("cg", par), 13 * HT, bf16), (("cq", par), 9 * HT, bf16)]
    scratch = [pltpu.VMEM((n, T), dt) for (_, n, dt) in names]
    nstep = BH // hb; grp = [(a, b - a) for a, b in zip((0,) + cut, cut + (hb,))]; ng = len(grp)
    obufs = [pltpu.VMEM((2, hb, r, D), bf16) for r in (Sq, Sq, Sk, Sk)]
    def kern(q_ref, k_ref, v_ref, g_ref, o_hbm, dq_hbm, dk_hbm, dv_hbm, sem, *scr):
        ob, scr = scr[:4], scr[4:]
        o_ref, dq_ref, dk_ref, dv_ref = range(4)
        step = pl.program_id(0); slot = step & 1
        def ocopy(a, gi, sp):
            dst = (o_hbm, dq_hbm, dk_hbm, dv_hbm)[a].at[pl.ds(sp * hb + grp[gi][0], grp[gi][1])]
            return pltpu.make_async_copy(ob[a].at[sp & 1, pl.ds(*grp[gi])], dst, sem.at[ng * a + gi, sp & 1])
        def obuf(a, h): return ob[a], h
        sc = {n[0]: r for n, r in zip(names, scr)}
        z = jax.lax.shift_right_logical(pl.program_id(0), 24)
        zv = jnp.full((8, T), z, i32)
        st = [dict() for _ in range(hb)]
        toks = []; marks = []; win = [0, 0]; pend = []; fin = []
        def drain(x):
            lim = len(toks) - (lag if fin else lag0)
            if not (pend and pend[0][0] <= lim): return x
            y = pltpu.bitcast(x[:8], i32)
            while pend and pend[0][0] <= lim: y = y | (pltpu.bitcast(pend.pop(0)[1], i32) & zv)
            return jnp.concatenate([pltpu.bitcast(y, u32), x[8:]], axis=0)
        def tie(m8, f):
            if win[1] <= win[0]: return m8
            ti = min(win[0] + int((win[1] - win[0]) * f), len(toks) - 1); x, r = toks[ti]
            y = pltpu.bitcast(m8, i32) | (pltpu.bitcast(x[r * 8:r * 8 + 8], i32) & zv)
            return pltpu.bitcast(y, m8.dtype)
        def addtoks(x): toks.extend((x, r) for r in range(x.shape[0] // 8))
        def rows(ref, h, r0, n, f=None, dep=False):
            x = ref.bitcast(u32)[h, r0 // 2:(r0 + n) // 2, :]
            if f is not None: x = jnp.concatenate([tie(x[:8], f), x[8:]], axis=0)
            return pltpu.bitcast(drain(x) if dep else x, bf16)
        def sput(key, r0, x):
            r = sc[key]
            if x.dtype == bf16: r.bitcast(u32)[r0 // 2:(r0 + x.shape[0]) // 2, :] = pltpu.bitcast(x, u32)
            else: r[r0:r0 + x.shape[0], :] = x.astype(r.dtype)
        def sget(key, r0, n, dep=False):
            r = sc[key]
            if r.dtype == f32: return r[pl.ds(pl.multiple_of(z + r0, 8), n), :]
            x = r.bitcast(u32)[pl.ds(pl.multiple_of(z + r0 // 2, 8), n // 2), :]
            return pltpu.bitcast(drain(x) if dep else x, bf16)
        def outT(ref, h, r0, x):
            y = pltpu.bitcast(x.astype(bf16).T, u32)
            pend.append((len(toks), y[HT - 8:]))
            buf, hl = obuf(ref, h)
            buf.bitcast(u32)[slot, hl, r0 // 2:(r0 + T) // 2, :] = y
        def colsum(x): return jnp.sum(x, axis=0, keepdims=True)
        def S(h, j):
            qs = rows(q_ref, h, j * T, T)
            ms = []
            for i in range(nc):
                x = dot(rows(k_ref, h, i * ck, ck, dep=True), qs, NT)
                if i == 0: addtoks(x)
                x = x * c
                sput(("s", h % 2, j, i), 0, x)
                ms.append(x.reshape(ck // 8, 8, T).max(0))
            m = jnp.max(functools.reduce(jnp.maximum, ms), axis=0, keepdims=True)
            st[h]["m", j] = jnp.broadcast_to(m, (8, T))
        def ex(h, j, r0, n, m):
            s = sget(("s", h % 2, j, r0 // ck), r0 % ck, n)
            return jnp.exp2(s.reshape(n // 8, 8, T) - m[None])
        def L(h, j):
            m = st[h]["m", j]; n = Sk // gl
            ls = [ex(h, j, i * gl, gl, tie(m, i / n)).sum(0) for i in range(n)]
            st[h]["m", j] = m + jnp.log2(jnp.broadcast_to(colsum(tsum(ls)), (8, T)))
        def Xs(h):
            m = st[h]["m", 2]; n = Sk // gl; ls = []
            for i in range(n):
                e = ex(h, 2, i * gl, gl, tie(m, i / n))
                sput(("ps", h % 2, i * gl // ck), i * gl % ck, e.reshape(gl, T)); ls.append(e.sum(0))
            st[h]["r"] = 1.0 / colsum(tsum(ls))
        def Xp(h):
            m0 = st[h]["m", 0]; m1 = st[h]["m", 1]; n = KH // gx
            for t in range(n):
                ms = [tie(m0, t / n), tie(m1, t / n)]
                b = [ex(h, j, a * KH + t * gx, gx, ms[j]).reshape(gx, T) for a in range(2) for j in range(2)]
                i, o = divmod(t * gx, T)
                for r, x in enumerate(bcomb(*b) + [b[1], b[2]]): sput(("pp", h % 2, i), r * T + o, x)
        def Tr(ref, nm, h):
            for i in range(4):
                for a in range(2): sput((nm, h % 2, i), a * T, rows(ref, h, a * KH + i * T, T, (2 * i + a) / 8).T)
        def Ac(nm, h):
            for i in range(4):
                for o in range(0, HT, 16):
                    f = (i * HT + o) / (4 * HT)
                    xs = [tie(sget((nm, h % 2, i), r0 + o, 16), f).astype(f32) for r0 in (0, T, HT, T + HT)]
                    cs = [x for x in acomb(*xs) if x is not None]
                    for r, x in enumerate(cs): sput((nm + "c", h % 2, i), r * HT + o, x)
        AOFF = [("c", 0), ("c", HT), ("", 0), ("", 3 * HT), ("c", 2 * HT), ("c", 3 * HT), ("c", 4 * HT)]
        def Cmb(ref, nm, h, mul):
            ts = [rows(ref, h, j * T, T, j / 3).T.astype(f32) for j in range(3)]
            if mul is not None: ts = [x * mul for x in ts]
            cs = ccomb(ts[0][:HT], ts[1][:HT], ts[0][HT:], ts[1][HT:]) + [ts[2] * st[h]["r"]]
            if mul is None: cs += [None, ts[0][HT:], ts[1][:HT], ts[2]]
            for r, x in enumerate(cs):
                if x is not None: sput((nm, h % 2), r * HT, x)
        def fwdp(h, an, bn):
            M = {}
            for r in (2, 4, 0, 6, 3, 1, 5):
                ps = [dot(sget((an + AOFF[r][0], h % 2, i), AOFF[r][1], HT, True), sget((bn, h % 2, i), r * T, T)) for i in range(4)]
                addtoks(ps[0]); M[r] = tsum(ps)
            return [[((M[0] - M[4]) + M[6]) + M[3], M[2] + M[4]], [M[3] + M[1], ((M[2] + M[0]) - M[1]) + M[5]]]
        def fwds(h, an, bn):
            ps = [dot(sget((an, h % 2, t % 4), t // 4 * T, T, True), sget((bn, h % 2, t // 2), t % 2 * T, T)) for t in range(8)]
            addtoks(ps[0]); addtoks(ps[4])
            return tsum(ps)
        def Op(h):
            C = fwdp(h, "av", "pp")
            G = [[sget(("cg", h % 2), o * HT, HT).astype(f32) for o in row] for row in ((6, 10), (9, 5))]
            for j in range(2):
                st[h]["d", j] = colsum(G[0][j] * C[0][j] + G[1][j] * C[1][j])
                outT(o_ref, h, j * T, jnp.concatenate([C[0][j], C[1][j]], axis=0))
        def Os(h):
            ot = fwds(h, "av", "ps") * st[h]["r"]
            st[h]["d", 2] = colsum(sget(("cg", h % 2), 11 * HT, T).astype(f32) * ot)
            outT(o_ref, h, 2 * T, ot)
        def Qp(h):
            C = fwdp(h, "ak", "dp")
            for j in range(2): outT(dq_ref, h, j * T, jnp.concatenate([C[0][j], C[1][j]], axis=0) * scale)
        def Qs(h): outT(dq_ref, h, 2 * T, fwds(h, "ak", "ds") * (st[h]["r"] * scale))
        def Pp(h):
            gs = [rows(g_ref, h, j * T, T) for j in range(2)]
            for s in range(2):
                p = [dot(rows(v_ref, h, a * KH + s * ck, ck, dep=True), gs[j], NT) for a in range(2) for j in range(2)]
                addtoks(p[0])
                for u in range(2):
                    i = 2 * s + u
                    d = [sget(("pp", h % 2, i), r * T, T).astype(f32) * (p[n][u * T:(u + 1) * T] - st[h]["d", n % 2])
                         for n, r in enumerate((1, 7, 8, 4))]
                    for r, x in enumerate(bcomb(*d)): sput(("dp", h % 2, i), r * T, x)
        def Ps(h):
            g2 = rows(g_ref, h, 2 * T, T)
            for i in range(nc):
                p = dot(rows(v_ref, h, i * ck, ck, dep=True), g2, NT)
                if i == 0: addtoks(p)
                sput(("ds", h % 2, i), 0, sget(("ps", h % 2, i), 0, ck).astype(f32) * (p - st[h]["d", 2]))
        def bwd(h, cn, bn, sn, out_ref):
            cnt = 0
            for i in range(4):
                N = {}
                for r in (4, 6, "a1", 2, 0, 5, "a0", 1, 3):
                    if isinstance(r, str):
                        t = int(r[1]) * 4 + i; w = sget((sn, h % 2, t // 2), t % 2 * T, T)
                        x = dot(sget((cn, h % 2), 7 * HT, T), w, NT); js = [x[:HT], x[HT:]]
                        N[r] = js
                    else:
                        N[r] = dot(sget((cn, h % 2), r * HT, HT, True), sget((bn, h % 2, i), r * T, T), NT); js = [N[r]]
                    for x in js:
                        if cnt % 4 == 0: addtoks(x)
                        cnt += 1
                d01 = (N[4] + N[6]) + N["a1"][0]
                d00 = (((N[4] + N[2]) + N[0]) - N[5]) + N["a0"][0]
                d10 = (N[5] + N["a0"][1]) + N[1]
                d11 = (((N["a1"][1] - N[6]) + N[0]) + N[1]) + N[3]
                outT(out_ref, h, i * T, jnp.concatenate([d00, d10], axis=0))
                outT(out_ref, h, KH + i * T, jnp.concatenate([d01, d11], axis=0))
        def Ky(h):
            for i in range(4):
                N = {}
                for n, r in enumerate((4, 6, 2, 0, 5, 1, 3)):
                    N[r] = dot(sget(("cq", h % 2), r * HT, HT, True), sget(("dp", h % 2, i), r * T, T), NT)
                    if (7 * i + n) % 4 == 0: addtoks(N[r])
                lo = jnp.concatenate([((N[4] + N[2]) + N[0]) - N[5], N[5] + N[1]], axis=0)
                hi = jnp.concatenate([N[4] + N[6], ((N[0] - N[6]) + N[1]) + N[3]], axis=0)
                sput(("s", h % 2, 0, i // 2), i % 2 * T, lo.T); sput(("s", h % 2, 0, 2 + i // 2), i % 2 * T, hi.T)
        def Kz(h):
            w = sget(("cq", h % 2), 7 * HT, T)
            for i in range(nc):
                x = dot(sget(("ds", h % 2, i), 0, ck, True), w, NT); a = sget(("s", h % 2, 0, i), 0, ck)
                if i == nc - 1:
                    y = pltpu.bitcast(a[kt:kt + 8], i32)
                    while pend: y = y | (pltpu.bitcast(pend.pop(0)[1], i32) & zv)
                    a = jnp.concatenate([a[:kt], pltpu.bitcast(y, f32), a[kt + 8:]], axis=0)
                x = x + a
                buf, hl = obuf(dk_ref, h)
                buf[slot, hl, i * ck:(i + 1) * ck, :] = x.astype(bf16)
        F = dict(Ky=Ky, Kz=Kz, Sa=lambda h: S(h, 0), Sb=lambda h: S(h, 1), Sc=lambda h: S(h, 2), Xs=Xs, Xp=Xp, Op=Op, Os=Os, Qp=Qp, Qs=Qs,
                 Pp=Pp, Ps=Ps, V=lambda h: bwd(h, "cg", "pp", "ps", dv_ref), K=lambda h: bwd(h, "cq", "dp", "ds", dk_ref),
                 La=lambda h: L(h, 0), Lb=lambda h: L(h, 1), Av=lambda h: Ac("av", h), Ak=lambda h: Ac("ak", h),
                 Tv=lambda h: Tr(v_ref, "av", h), Tk=lambda h: Tr(k_ref, "ak", h),
                 Cg=lambda h: Cmb(g_ref, "cg", h, None), Cq=lambda h: Cmb(q_ref, "cq", h, scale))
        done = set()
        for h0 in range(hb):
            for tok in (PRO + " " + REST if h0 == 0 else LAST if h0 == hb - 1 else HEAD + " " + REST).split():
                if tok == "F": fin.append(1); continue
                tok, _, w = tok.partition("@"); nm, h = tok[:-1], h0 + int(tok[-1])
                if h >= hb: continue
                assert (nm, h) not in done; done.add((nm, h))
                if w:
                    w, _, mg = w.partition("/")
                    win[:] = [marks[-int(w)], len(toks) - 8 * int(mg or 0)] if int(w) else [0, 0]
                else: marks.append(len(toks))
                if nm == dat and h in cut:
                    assert all((x, y) in done for x in ("Os", "Op", "V", "K", "Qs", "Qp") for y in range(h))
                    for a in range(4): ocopy(a, cut.index(h), step).start()
                F[nm](h)
        assert len(done) == (len(F) - 2) * hb + (("Ky", hb - 1) in done) and all((dat, y) in done for y in cut)
        for a in (0, 3, 1, 2): ocopy(a, ng - 1, step).start()
        def waits(sp, carry):
            for a in range(4 * ng): ocopy(a // ng, a % ng, sp).wait()
            return carry
        jax.lax.fori_loop(jnp.maximum(step - 1, 0), jnp.where(step == nstep - 1, step + 1, step), waits, 0)
    qs = pl.BlockSpec((hb, Sq, D), lambda i: (i, 0, 0))
    ks = pl.BlockSpec((hb, Sk, D), lambda i: (i, 0, 0))
    sq = jax.ShapeDtypeStruct((BH, Sq, D), bf16); sk = jax.ShapeDtypeStruct((BH, Sk, D), bf16)
    o, dq, dk, dv = pl.pallas_call(kern, grid=(BH // hb,), in_specs=[qs, ks, ks, qs], out_specs=[pl.BlockSpec(memory_space=pl.ANY)] * 4,
        scratch_shapes=[pltpu.SemaphoreType.DMA((4 * ng, 2))] + obufs + scratch, out_shape=[sq, sq, sk, sk],
        compiler_params=pltpu.CompilerParams(dimension_semantics=("arbitrary",), vmem_limit_bytes=100*1024*1024, disable_bounds_checks=True),
    )(q.reshape(BH, Sq, D), k.reshape(BH, Sk, D), v.reshape(BH, Sk, D), g.reshape(BH, Sq, D))
    return o.reshape(q.shape), dq.reshape(q.shape), dk.reshape(k.shape), dv.reshape(k.shape)
```
